```python
import os as _os
_os.environ.setdefault("JAX_PLATFORMS", "cpu")
import jax
import jax.numpy as jnp

def _softmax(x, axis=-1):
    return jax.nn.softmax(x, axis=axis)
def _gelu(x):
    return jax.nn.gelu(x, approximate=True)
def _silu(x):
    return jax.nn.silu(x)
def _sigmoid(x):
    return jax.nn.sigmoid(x)
def _layernorm(x, axis=-1, eps=1e-5):
    m = jnp.mean(x, axis=axis, keepdims=True)
    v = jnp.var(x, axis=axis, keepdims=True)
    return (x - m) / jnp.sqrt(v + eps)
def _scatter_add(tgt, idx, src, axis=0):
    return tgt.at[idx].add(src)
def _segment_sum(src, seg, n):
    return jax.ops.segment_sum(src, seg, n)
class _Rng:
    def __init__(self, key):
        self._k = key
    def _next(self):
        self._k, sub = jax.random.split(self._k)
        return sub
    def normal(self, shape):
        return jax.random.normal(self._next(), shape, dtype=jnp.bfloat16)
    def randint(self, lo, hi, shape):
        return jax.random.randint(self._next(), shape, lo, hi, dtype=jnp.int32)
    def uniform(self, shape, lo=0.0, hi=1.0):
        return jax.random.uniform(self._next(), shape, jnp.bfloat16, lo, hi)
    def permutation(self, n):
        return jax.random.permutation(self._next(), n)


kernel_name = 'parallel_sum__softmax_full_mha__swiglu_ffn__prompt'

def setup_inputs():
    _rng = _Rng(jax.random.key(int.from_bytes(__import__("os").urandom(4), "little")))
    _w = (lambda a: (lambda t: t.astype(jnp.bfloat16) if jnp.issubdtype(t.dtype, jnp.floating) else t)(jnp.asarray(a)))
    def _A_setup():
        B, S, D = 1, 2048, 640
        return {
            "x": _w((lambda *s: _rng.normal(s) * 0.05)(B, S, D)),
            "wqkv": _w((lambda *s: _rng.normal(s) * 0.1)(D, 3 * D)),
            "wo": _w((lambda *s: _rng.normal(s) * 0.05)(D, D)),
        }
    _A_in = _A_setup()

    def _B_setup():
        B, S, D, F = 1, 2048, 640, 1536
        return {
            "x": _w((lambda *s: _rng.normal(s) * 0.05)(B, S, D)),
            "w_gate": _w((lambda *s: _rng.normal(s) * 0.05)(D, F)),
            "w_up": _w((lambda *s: _rng.normal(s) * 0.05)(D, F)),
            "w_down": _w((lambda *s: _rng.normal(s) * 0.05)(F, D)),
        }
    _B_in = _B_setup()

    return {
        "A_x": _A_in["x"],
        "A_wqkv": _A_in["wqkv"],
        "A_wo": _A_in["wo"],
        "B_x": _B_in["x"],
        "B_w_gate": _B_in["w_gate"],
        "B_w_up": _B_in["w_up"],
        "B_w_down": _B_in["w_down"],
    }

def reference(A_x, A_wqkv, A_wo, B_x, B_w_gate, B_w_up, B_w_down):
    def _A_ref(x, wqkv, wo):
        B, S, D = x.shape
        H = 32; Dh = D // H
        qkv = (lambda x, *d: x.transpose(*d))((x @ wqkv).reshape(B, S, 3, H, Dh), 2, 0, 3, 1, 4)
        q, k, v = qkv[0], qkv[1], qkv[2]
        scale = Dh ** -0.5
        scores = jnp.einsum("bhqd,bhkd->bhqk", q, k) * scale
        p = _softmax(scores, axis=-1)
        o = jnp.einsum("bhqk,bhkd->bhqd", p, v)
        return (lambda x, *d: x.transpose(*d))(o, 0, 2, 1, 3).reshape(B, S, D) @ wo

    def _B_ref(x, w_gate, w_up, w_down):
        g = _silu(x @ w_gate)
        u = x @ w_up
        return (g * u) @ w_down

    x = A_x
    xn = _layernorm(x, axis=-1)
    return x + _A_ref(xn, A_wqkv, A_wo) + _B_ref(xn, B_w_gate, B_w_up, B_w_down)
```

```python
import jax
import jax.numpy as jnp
from jax import lax
import jax.experimental.pallas as pl
import jax.experimental.pallas.tpu as pltpu

S, D, H, F = 2048, 640, 32, 1536
DH = D // H
HPG = 128 // DH
NG = -(-H // HPG)
BQ = 1024
NB = S // BQ
CH = 128
LAG = 2
UP = 2
RP = 512
RF = 512
VR = 32
QSCALE = DH ** -0.5 * 1.4426950408889634

_NT = (((1,), (1,)), ((), ()))


def _kernel(x_hbm, wqkv_hbm, wo_hbm, wg_hbm, wu_hbm, wd_hbm, o_hbm,
            x_ref, wqkv_ref, wo_ref, wg_ref, wu_ref, wd_ref, ob_ref,
            xn_ref, k_ref, qt_ref, vt_ref, s_ref, ot_ref, wqt_ref, wvt_ref,
            in_sem, out_sem):
    f32, bf16 = jnp.float32, jnp.bfloat16
    NP = S // RP

    def x_copy(b):
        r = pl.ds(b * RP, RP)
        return pltpu.make_async_copy(x_hbm.at[r, :], x_ref.at[r, :], in_sem.at[b])

    def wqkv_copy(j):
        c = pl.ds(j * D, D)
        return pltpu.make_async_copy(wqkv_hbm.at[:, c], wqkv_ref.at[:, c], in_sem.at[NP + j])

    late = [pltpu.make_async_copy(src, dst, in_sem.at[NP + 3 + j]) for j, (src, dst) in enumerate(
        ((wg_hbm, wg_ref), (wu_hbm, wu_ref), (wd_hbm, wd_ref), (wo_hbm, wo_ref)))]

    rows = lax.broadcasted_iota(jnp.int32, (128, BQ), 0)
    ninf = jnp.full((8, BQ), -jnp.inf, f32)
    tail = (lax.broadcasted_iota(jnp.int32, (VR - DH, RP), 0) == 0).astype(f32)

    def norm(b):
        r = pl.ds(pl.multiple_of(b * RP, RP), RP)
        x = x_ref[r, :].astype(f32)
        xc = x - jnp.mean(x, axis=-1, keepdims=True)
        var = jnp.mean(xc * xc, axis=-1, keepdims=True)
        xn_ref[r, :] = (xc * lax.rsqrt(var + 1e-5)).astype(bf16)

    def project_k(b):
        r = pl.ds(pl.multiple_of(b * RP, RP), RP)
        k = jnp.dot(xn_ref[r, :], wqkv_ref[:, D:2 * D], preferred_element_type=f32).astype(bf16)
        k = jnp.concatenate([k, jnp.zeros((RP, 128), bf16)], axis=1)
        for g in range(NG):
            k_ref[g, r, :] = k[:, g * HPG * DH:g * HPG * DH + 128]

    def project_qv(b):
        r = pl.ds(pl.multiple_of(b * RP, RP), RP)
        xn = xn_ref[r, :]
        q_t = lax.dot_general(wqt_ref[...], xn, _NT, preferred_element_type=f32) * QSCALE
        q_t = jnp.concatenate([q_t, jnp.zeros((128, RP), f32)], axis=0)
        for g in range(NG):
            qt_ref[b * RP // BQ, g, :, pl.ds(pl.multiple_of(b * RP % BQ, RP), RP)] = (
                q_t[g * HPG * DH:g * HPG * DH + 128, :].astype(bf16))
        v_t = lax.dot_general(wvt_ref[...], xn, _NT, preferred_element_type=f32)
        for h in range(H):
            vt_ref[h, :, r] = jnp.concatenate(
                [v_t[h * DH:(h + 1) * DH, :], tail], axis=0).astype(bf16)

    def masked_q(b, h):
        g = h // HPG
        lo = (h - g * HPG) * DH
        q = qt_ref[b, g].astype(f32)
        return jnp.where((rows >= lo) & (rows < lo + DH), q, 0.0).astype(bf16)

    def qk_chunk(h, qm, c, m):
        s = jnp.dot(k_ref[h // HPG, pl.ds(c * CH, CH), :], qm, preferred_element_type=f32)
        s_ref[pl.ds(c * CH, CH), :] = s
        return jnp.maximum(m, jnp.max(s.reshape(CH // 8, 8, BQ), axis=0))

    def pv_chunk(h, c, mb, acc):
        s = s_ref[pl.ds(c * CH, CH), :].reshape(CH // 8, 8, BQ)
        p = jnp.exp2(s - mb[None]).reshape(CH, BQ).astype(bf16)
        r = jnp.dot(vt_ref[h, :, pl.ds(c * CH, CH)], p, preferred_element_type=f32)
        return r if acc is None else acc + r

    def head(h, nxt, m):
        mb = jnp.broadcast_to(jnp.max(m, axis=0, keepdims=True), (8, BQ))
        if nxt is not None:
            qm = masked_q(*nxt)
        m, acc, seen = ninf, None, []
        for c in range(S // CH):
            mc = mb
            if nxt is not None and c >= LAG:
                mc = jnp.minimum(mb, jnp.maximum(mb, seen[c - LAG]))
            acc = pv_chunk(h, c, mc, acc)
            if nxt is not None:
                m = qk_chunk(nxt[1], qm, c, m)
                seen.append(m)
        return acc[0:DH, :] / acc[DH:DH + 1, :], m

    def pair(i, m, last=False):
        b = i // (H // 2)
        h = 2 * i - b * H
        o0, m = head(h, (b, h + 1), m)
        nb = (i + 1) // (H // 2)
        o1, m = head(h + 1, None if last else (nb, 2 * (i + 1) - nb * H), m)
        o = jnp.concatenate([o0, o1], axis=0)
        for j in range(BQ // RF):
            ot_ref[b * (BQ // RF) + j, pl.ds(pl.multiple_of(h * DH, 8), 2 * DH), :] = (
                o[:, j * RF:(j + 1) * RF])
        return m

    def pairs(i, m):
        for j in range(UP):
            m = pair(i * UP + j, m)
        return m

    def out_copy(i):
        r = pl.ds(pl.multiple_of(i * RF, RF), RF)
        return pltpu.make_async_copy(ob_ref.at[i], o_hbm.at[r, :], out_sem.at[i])

    x_copy(0).start()
    wqkv_copy(1).start()
    x_copy(0).wait()
    x_copy(1).start()
    norm(0)
    wqkv_copy(1).wait()
    wqkv_copy(0).start()
    wqkv_copy(2).start()
    x_copy(1).wait()
    project_k(0)
    norm(1)
    wqkv_copy(0).wait()
    wqkv_copy(2).wait()
    for b in range(2, NP):
        x_copy(b).start()
    project_k(1)
    wqt_ref[...] = wqkv_ref[:, 0:D].T
    wvt_ref[...] = wqkv_ref[:, 2 * D:3 * D].T
    for b in range(2, NP):
        x_copy(b).wait()

    @pl.loop(0, NP - 2)
    def _(b):
        project_qv(b)
        norm(b + 2)
        project_k(b + 2)

    for b in range(NP - 2, NP):
        project_qv(b)

    qm = masked_q(0, 0)
    m = ninf
    for c in range(S // CH):
        m = qk_chunk(0, qm, c, m)

    for c in late:
        c.start()
    n_pairs = NB * H // 2
    n_loop = (n_pairs - 1) // UP
    m = lax.fori_loop(0, n_loop, pairs, m)
    for c in late:
        c.wait()
    for i in range(n_loop * UP, n_pairs):
        m = pair(i, m, last=i == n_pairs - 1)

    @pl.loop(0, S // RF)
    def _(i):
        r = pl.ds(pl.multiple_of(i * RF, RF), RF)
        xn = xn_ref[r, :]
        g = jnp.dot(xn, wg_ref[...], preferred_element_type=f32)
        u = jnp.dot(xn, wu_ref[...], preferred_element_type=f32)
        hid = (g * jax.nn.sigmoid(g) * u).astype(bf16)
        out = jnp.dot(hid, wd_ref[...], preferred_element_type=f32)
        out += jnp.dot(ot_ref[i].astype(bf16).T, wo_ref[...], preferred_element_type=f32)
        ob_ref[i] = (out + x_ref[r, :].astype(f32)).astype(ob_ref.dtype)
        out_copy(i).start()

    for i in range(S // RF):
        out_copy(i).wait()


@jax.jit
def pallas_parallel_sum__softmax_full_mha__swiglu_ffn__prompt_kernel(
    A_x: jax.Array,
    A_wqkv: jax.Array,
    A_wo: jax.Array,
    B_x: jax.Array,
    B_w_gate: jax.Array,
    B_w_up: jax.Array,
    B_w_down: jax.Array,
):
    del B_x
    args = (A_x.reshape(S, D), A_wqkv, A_wo, B_w_gate, B_w_up, B_w_down)
    out = pl.pallas_call(
        _kernel,
        in_specs=[pl.BlockSpec(memory_space=pl.ANY)] * len(args),
        out_specs=pl.BlockSpec(memory_space=pl.ANY),
        out_shape=jax.ShapeDtypeStruct((S, D), A_x.dtype),
        scratch_shapes=[pltpu.VMEM(a.shape, a.dtype) for a in args] + [
            pltpu.VMEM((S // RF, RF, D), A_x.dtype),
            pltpu.VMEM((S, D), jnp.bfloat16),
            pltpu.VMEM((NG, S, 128), jnp.bfloat16),
            pltpu.VMEM((NB, NG, 128, BQ), jnp.bfloat16),
            pltpu.VMEM((H, VR, S), jnp.bfloat16),
            pltpu.VMEM((S, BQ), jnp.float32),
            pltpu.VMEM((S // RF, D, RF), jnp.float32),
            pltpu.VMEM((D, D), jnp.bfloat16),
            pltpu.VMEM((D, D), jnp.bfloat16),
            pltpu.SemaphoreType.DMA((S // RP + 7,)),
            pltpu.SemaphoreType.DMA((S // RF,)),
        ],
        compiler_params=pltpu.CompilerParams(vmem_limit_bytes=100 * 2**20),
        name="mha_swiglu_block",
    )(*args)
    return out.reshape(A_x.shape)
```
